```python
import os as _os
_os.environ.setdefault("JAX_PLATFORMS", "cpu")
import jax
import jax.numpy as jnp

def _softmax(x, axis=-1):
    return jax.nn.softmax(x, axis=axis)
def _gelu(x):
    return jax.nn.gelu(x, approximate=True)
def _silu(x):
    return jax.nn.silu(x)
def _sigmoid(x):
    return jax.nn.sigmoid(x)
def _layernorm(x, axis=-1, eps=1e-5):
    m = jnp.mean(x, axis=axis, keepdims=True)
    v = jnp.var(x, axis=axis, keepdims=True)
    return (x - m) / jnp.sqrt(v + eps)
def _scatter_add(tgt, idx, src, axis=0):
    return tgt.at[idx].add(src)
def _segment_sum(src, seg, n):
    return jax.ops.segment_sum(src, seg, n)
class _Rng:
    def __init__(self, key):
        self._k = key
    def _next(self):
        self._k, sub = jax.random.split(self._k)
        return sub
    def normal(self, shape):
        return jax.random.normal(self._next(), shape, dtype=jnp.bfloat16)
    def randint(self, lo, hi, shape):
        return jax.random.randint(self._next(), shape, lo, hi, dtype=jnp.int32)
    def uniform(self, shape, lo=0.0, hi=1.0):
        return jax.random.uniform(self._next(), shape, jnp.bfloat16, lo, hi)
    def permutation(self, n):
        return jax.random.permutation(self._next(), n)


kernel_name = 'standalone__detection_seg_fpn_lateral__vision'

def setup_inputs():
    _rng = _Rng(jax.random.key(int.from_bytes(__import__("os").urandom(4), "little")))
    _w = (lambda a: (lambda t: t.astype(jnp.bfloat16) if jnp.issubdtype(t.dtype, jnp.floating) else t)(jnp.asarray(a)))
    H = W = (256 // 2) * 2
    C = 384
    k = 1
    return {
        "c_fine": _w((lambda *s: _rng.normal(s) * 0.05)(1, H, W, C)),
        "p_coarse": _w((lambda *s: _rng.normal(s) * 0.05)(1, H // 2, W // 2, C)),
        "w_lat": _w((lambda *s: _rng.normal(s) * 0.05)(C, C)),
        "w_out": _w((lambda *s: _rng.normal(s) * 0.05)(k, k, C, C)),
    }

def reference(c_fine, p_coarse, w_lat, w_out):
    B, H, W, C = c_fine.shape
    k = 1
    lat = jnp.einsum("bhwc,cd->bhwd", c_fine, w_lat)
    up = jnp.repeat(jnp.repeat(p_coarse, 2, axis=1), 2, axis=2)
    m = lat + up
    pad = k // 2
    mp = jnp.pad(m, ((0, 0), (pad, pad), (pad, pad), (0, 0)))
    o = None
    for di in range(k):
        for dj in range(k):
            t = jnp.einsum("bhwc,cd->bhwd", mp[:, di:di + H, dj:dj + W, :], w_out[di, dj])
            o = t if o is None else o + t
    return o
```

```python
import jax
import jax.numpy as jnp
from jax import lax
import jax.experimental.pallas as pl
import jax.experimental.pallas.tpu as pltpu

_G = 32
_A = 4
_B = 4
_BLK = 64
_NM = _A * _B
_SUB = 4
_S_TRANS = 35
_TAIL_G = 8


def _kernel(c_hbm, p_hbm, wl_hbm, wo_hbm, o_hbm,
            cbuf, pbuf, obuf, wl, wo, wc, csem, psem, osem, wsem):
    C = wl.shape[-1]
    gs = _G // _SUB
    m_trans = _S_TRANS // _SUB

    def c_copy(m):
        return pltpu.make_async_copy(
            c_hbm.at[:, m // _B, :, m % _B], cbuf.at[m], csem.at[m])

    def p_copy(m):
        return pltpu.make_async_copy(p_hbm.at[:, m], pbuf.at[m], psem.at[m])

    def p_last_head():
        n = _G - _TAIL_G
        return pltpu.make_async_copy(
            p_hbm.at[pl.ds(0, n), _NM - 1], pbuf.at[_NM - 1, pl.ds(0, n)],
            psem.at[_NM - 1])

    def p_last_tail():
        n = _G - _TAIL_G
        return pltpu.make_async_copy(
            p_hbm.at[pl.ds(n, _TAIL_G), _NM - 1],
            pbuf.at[_NM - 1, pl.ds(n, _TAIL_G)], psem.at[_NM])

    def o_copy(m, par):
        return pltpu.make_async_copy(
            obuf.at[m, :, par], o_hbm.at[:, m // _B, par, m % _B],
            osem.at[m, par])

    wl_cp = pltpu.make_async_copy(wl_hbm, wl, wsem.at[0])
    wo_cp = pltpu.make_async_copy(wo_hbm, wo, wsem.at[1])
    wl_cp.start()
    wo_cp.start()
    for m in range(_NM):
        if m < _NM - 1:
            p_copy(m).start()
            c_copy(m).start()
        else:
            c_copy(m).start()
            p_last_head().start()
            p_last_tail().start()
    wl_cp.wait()
    wo_cp.wait()
    wc[...] = jnp.dot(wl[...], wo[...],
                      preferred_element_type=jnp.float32).astype(wc.dtype)

    def body(s, carry):
        m = s // _SUB
        j = s % _SUB

        @pl.when(jnp.logical_and(j == 0, s <= _S_TRANS))
        def _():
            p_copy(m).wait()
            c_copy(m).wait()

        @pl.when(s == _S_TRANS)
        def _():
            for mm in range(m_trans + 1, _NM):
                c_copy(mm).wait()
                if mm < _NM - 1:
                    p_copy(mm).wait()
                else:
                    p_last_head().wait()
            for mm in range(m_trans):
                o_copy(mm, 0).start()
                o_copy(mm, 1).start()
            p_last_tail().wait()

        g0 = pl.multiple_of(j * gs, gs)
        pv = pbuf[m, pl.ds(g0, gs)].reshape(gs * (_BLK // 2), C)
        q = jnp.dot(pv, wo[...], preferred_element_type=jnp.float32)
        qq = pltpu.pack_elementwise([q, q], packed_dtype=jnp.bfloat16)
        up = pltpu.bitcast(qq, jnp.bfloat16).astype(jnp.float32)
        up = up.reshape(gs, 1, _BLK, C)
        cv = cbuf[m, pl.ds(g0, gs)].reshape(gs * 2 * _BLK, C)
        acc = jnp.dot(cv, wc[...], preferred_element_type=jnp.float32)
        acc = acc.reshape(gs, 2, _BLK, C)
        obuf[m, pl.ds(g0, gs)] = (acc + up).astype(obuf.dtype)

        @pl.when(jnp.logical_and(j == _SUB - 1, m >= m_trans))
        def _():
            o_copy(m, 0).start()
            o_copy(m, 1).start()
        return carry

    lax.fori_loop(0, _NM * _SUB, body, 0)
    for mm in range(_NM):
        o_copy(mm, 0).wait()
        o_copy(mm, 1).wait()


@jax.jit
def pallas_standalone__detection_seg_fpn_lateral__vision_kernel(
    c_fine: jax.Array,
    p_coarse: jax.Array,
    w_lat: jax.Array,
    w_out: jax.Array,
):
    Bn, H, W, C = c_fine.shape
    assert (Bn, H, W) == (1, _G * _A * 2, _B * _BLK)
    dt = c_fine.dtype
    c6 = c_fine.reshape(_G, _A, 2, _B, _BLK, C)
    p4 = p_coarse.reshape(_G, _NM, _BLK // 2, C)
    wo2 = w_out.reshape(C, C)
    out = pl.pallas_call(
        _kernel,
        in_specs=[pl.BlockSpec(memory_space=pl.ANY)] * 4,
        out_specs=pl.BlockSpec(memory_space=pl.ANY),
        out_shape=jax.ShapeDtypeStruct((_G, _A, 2, _B, _BLK, C), dt),
        scratch_shapes=[
            pltpu.VMEM((_NM, _G, 2, _BLK, C), dt),
            pltpu.VMEM((_NM, _G, _BLK // 2, C), dt),
            pltpu.VMEM((_NM, _G, 2, _BLK, C), dt),
            pltpu.VMEM((C, C), dt),
            pltpu.VMEM((C, C), dt),
            pltpu.VMEM((C, C), dt),
            pltpu.SemaphoreType.DMA((_NM,)),
            pltpu.SemaphoreType.DMA((_NM + 1,)),
            pltpu.SemaphoreType.DMA((_NM, 2)),
            pltpu.SemaphoreType.DMA((2,)),
        ],
        compiler_params=pltpu.CompilerParams(
            vmem_limit_bytes=126 * 1024 * 1024),
    )(c6, p4, w_lat, wo2)
    return out.reshape(Bn, H, W, C)
```

```python
import jax
import jax.numpy as jnp
from jax import lax
import jax.experimental.pallas as pl
import jax.experimental.pallas.tpu as pltpu

_G = 64
_A = 2
_B = 2
_BLK = 128
_GS = 4
_SUB = _G // _GS
_NS = _A * _B * _SUB
_LANE = 128

_C_BOUNDS = (0, 1, 2, 4, 8, 12, 16, 24, 32, 48, 64)
_P_BOUNDS = (0, 4, 16, 32, 48, 62, 64)
_W_BOUNDS = (0, 16, 32, 48, 56, 60, 64)
_S_TRANS = 37
_W_SPLIT = (40, 48, 40)


def _pairs(b):
    return list(zip(b[:-1], b[1:]))


def _box(s0, s1):
    m = s0 // _SUB
    assert (s1 - 1) // _SUB == m
    g0 = (s0 % _SUB) * _GS
    return pl.ds(g0, (s1 - s0) * _GS), m // _B, m % _B


_C_CH = _pairs(_C_BOUNDS)
_P_CH = _pairs(_P_BOUNDS)
_W_CH = _pairs(_W_BOUNDS)
_READS = sorted(
    [("p", i, r) for i, r in enumerate(_P_CH[:-1])]
    + [("c", i, r) for i, r in enumerate(_C_CH)],
    key=lambda t: (t[2][0], t[0] != "p"))
_TAIL = ("p", len(_P_CH) - 1, _P_CH[-1])


def _kernel(c_hbm, p_hbm, wl_hbm, wo_hbm, o_hbm,
            cbuf, pbuf, obuf, wl, wo, wc, up_ref, csem, psem, osem, wsem):
    C = wl.shape[-1]
    n = _GS * _BLK // 2

    def rd(kind, i, r):
        g, a, b = _box(*r)
        if kind == "c":
            return pltpu.make_async_copy(
                c_hbm.at[g, a, :, b], cbuf.at[g, a, :, b], csem.at[i])
        return pltpu.make_async_copy(
            p_hbm.at[g, a, b], pbuf.at[g, a, b], psem.at[i])

    def wr(u):
        g, a, b = _box(*_W_CH[u])
        cps = []
        for par in range(2):
            r0 = 0
            for k, rows in enumerate(_W_SPLIT):
                idx = (g, a, par, b, pl.ds(r0, rows))
                cps.append(pltpu.make_async_copy(
                    obuf.at[idx], o_hbm.at[idx],
                    osem.at[u, par * len(_W_SPLIT) + k]))
                r0 += rows
        return cps

    wl_cp = pltpu.make_async_copy(wl_hbm, wl, wsem.at[0])
    wo_cp = pltpu.make_async_copy(wo_hbm, wo, wsem.at[1])
    wl_cp.start()
    wo_cp.start()
    for t in _READS + [_TAIL]:
        rd(*t).start()
    wl_cp.wait()
    wo_cp.wait()
    wc[...] = jnp.dot(wl[...], wo[...],
                      preferred_element_type=jnp.float32).astype(wc.dtype)

    def body(s, carry):
        m = s // _SUB
        a = m // _B
        b = m % _B
        g0 = pl.multiple_of((s % _SUB) * _GS, _GS)

        for s0 in sorted({t[2][0] for t in _READS if t[2][0] < _S_TRANS}):
            @pl.when(s == s0)
            def _(s0=s0):
                for t in _READS:
                    if t[2][0] == s0:
                        rd(*t).wait()

        @pl.when(s == _S_TRANS)
        def _():
            for t in _READS:
                if t[2][0] >= _S_TRANS:
                    rd(*t).wait()
            for u, (_, u1) in enumerate(_W_CH):
                if u1 <= _S_TRANS:
                    for cp in wr(u):
                        cp.start()
            rd(*_TAIL).wait()

        pv = pbuf[pl.ds(g0, _GS), a, b].reshape(n, C)
        q = jnp.dot(pv, wo[...], preferred_element_type=jnp.float32)
        for k in range(C // _LANE):
            qk = q[:, k * _LANE:(k + 1) * _LANE]
            up_ref[k, pl.ds(0, n, stride=2), :] = qk
            up_ref[k, pl.ds(1, n, stride=2), :] = qk
        up = jnp.concatenate([up_ref[k] for k in range(C // _LANE)], axis=1)
        up = up.reshape(_GS, 1, _BLK, C)

        cv = cbuf[pl.ds(g0, _GS), a, :, b].reshape(_GS * 2 * _BLK, C)
        acc = jnp.dot(cv, wc[...], preferred_element_type=jnp.float32)
        acc = acc.reshape(_GS, 2, _BLK, C)
        obuf[pl.ds(g0, _GS), a, :, b] = (acc + up).astype(obuf.dtype)

        for u, (_, u1) in enumerate(_W_CH):
            if u1 > _S_TRANS:
                @pl.when(s == u1 - 1)
                def _(u=u):
                    for cp in wr(u):
                        cp.start()
        return carry

    lax.fori_loop(0, _NS, body, 0)
    for u in range(len(_W_CH)):
        for cp in wr(u):
            cp.wait()


@jax.jit
def pallas_standalone__detection_seg_fpn_lateral__vision_kernel(
    c_fine: jax.Array,
    p_coarse: jax.Array,
    w_lat: jax.Array,
    w_out: jax.Array,
):
    Bn, H, W, C = c_fine.shape
    assert (Bn, H, W) == (1, _G * _A * 2, _B * _BLK) and C % _LANE == 0
    dt = c_fine.dtype
    fine = (_G, _A, 2, _B, _BLK, C)
    coarse = (_G, _A, _B, _BLK // 2, C)
    out = pl.pallas_call(
        _kernel,
        in_specs=[pl.BlockSpec(memory_space=pl.ANY)] * 4,
        out_specs=pl.BlockSpec(memory_space=pl.ANY),
        out_shape=jax.ShapeDtypeStruct(fine, dt),
        scratch_shapes=[
            pltpu.VMEM(fine, dt),
            pltpu.VMEM(coarse, dt),
            pltpu.VMEM(fine, dt),
            pltpu.VMEM((C, C), dt),
            pltpu.VMEM((C, C), dt),
            pltpu.VMEM((C, C), dt),
            pltpu.VMEM((C // _LANE, _GS * _BLK, _LANE), jnp.float32),
            pltpu.SemaphoreType.DMA((len(_C_CH),)),
            pltpu.SemaphoreType.DMA((len(_P_CH),)),
            pltpu.SemaphoreType.DMA((len(_W_CH), 2 * len(_W_SPLIT))),
            pltpu.SemaphoreType.DMA((2,)),
        ],
        compiler_params=pltpu.CompilerParams(
            vmem_limit_bytes=126 * 1024 * 1024),
    )(c_fine.reshape(fine), p_coarse.reshape(coarse), w_lat,
      w_out.reshape(C, C))
    return out.reshape(Bn, H, W, C)
```

```python
import jax
import jax.numpy as jnp
from jax import lax
import jax.experimental.pallas as pl
import jax.experimental.pallas.tpu as pltpu

_G = 64
_A = 2
_B = 2
_BLK = 128
_GS = 4
_SUB = _G // _GS
_NS = _A * _B * _SUB
_LANE = 128

_C_BOUNDS = (0, 1, 2, 4, 6, 10, 16, 24, 32, 48, 64)
_P_BOUNDS = (0, 2, 6, 16, 32, 48, 62, 64)
_W_BOUNDS = (0, 16, 32, 48, 59, 64)
_S_TRANS = 37
_W_SPLIT = (48, 40, 40)


def _pairs(b):
    return list(zip(b[:-1], b[1:]))


def _box(s0, s1):
    m = s0 // _SUB
    assert (s1 - 1) // _SUB == m
    g0 = (s0 % _SUB) * _GS
    return pl.ds(g0, (s1 - s0) * _GS), m // _B, m % _B


_C_CH = _pairs(_C_BOUNDS)
_P_CH = _pairs(_P_BOUNDS)
_W_CH = _pairs(_W_BOUNDS)
_READS = sorted(
    [("p", i, r) for i, r in enumerate(_P_CH[:-1])]
    + [("c", i, r) for i, r in enumerate(_C_CH)],
    key=lambda t: (t[2][0], t[0] != "p"))
_TAIL = ("p", len(_P_CH) - 1, _P_CH[-1])
_WAIT_STEPS = sorted({t[2][0] for t in _READS if t[2][0] < _S_TRANS})
_WRITE_STEPS = [u1 for _, u1 in _W_CH if _S_TRANS < u1 < _NS]
_EVENTS = sorted({*_WAIT_STEPS, _S_TRANS, *_WRITE_STEPS})
_EVENTS_LO = sum(1 << e for e in _EVENTS if e < 32)
_EVENTS_HI = sum(1 << (e - 32) for e in _EVENTS if e >= 32)
assert _NS <= 64 and max(_EVENTS_LO, _EVENTS_HI) < 2 ** 31
assert _SUB == 16 and _B == 2 and _TAIL[2][0] >= _S_TRANS


def _kernel(c_hbm, p_hbm, wl_hbm, wo_hbm, o_hbm,
            cbuf, pbuf, obuf, wl, wo, wc, up_ref, csem, psem, osem, wsem):
    C = wl.shape[-1]
    n = _GS * _BLK // 2

    def rd(kind, i, r):
        g, a, b = _box(*r)
        if kind == "c":
            return pltpu.make_async_copy(
                c_hbm.at[g, a, :, b], cbuf.at[g, a, :, b], csem.at[i])
        return pltpu.make_async_copy(
            p_hbm.at[g, a, b], pbuf.at[g, a, b], psem.at[i])

    def wr(u):
        g, a, b = _box(*_W_CH[u])
        cps = []
        for par in range(2):
            r0 = 0
            for k, rows in enumerate(_W_SPLIT):
                idx = (g, a, par, b, pl.ds(r0, rows))
                cps.append(pltpu.make_async_copy(
                    obuf.at[idx], o_hbm.at[idx],
                    osem.at[u, par * len(_W_SPLIT) + k]))
                r0 += rows
        return cps

    wl_cp = pltpu.make_async_copy(wl_hbm, wl, wsem.at[0])
    wo_cp = pltpu.make_async_copy(wo_hbm, wo, wsem.at[1])
    wl_cp.start()
    wo_cp.start()
    for t in _READS + [_TAIL]:
        rd(*t).start()
    wl_cp.wait()
    wo_cp.wait()
    wc[...] = jnp.dot(wl[...], wo[...],
                      preferred_element_type=jnp.float32).astype(wc.dtype)

    def dma_bookkeeping(s):
        for s0 in _WAIT_STEPS:
            @pl.when(s == s0)
            def _(s0=s0):
                for t in _READS:
                    if t[2][0] == s0:
                        rd(*t).wait()

        @pl.when(s == _S_TRANS)
        def _():
            for t in _READS:
                if t[2][0] >= _S_TRANS:
                    rd(*t).wait()
            for u, (_, u1) in enumerate(_W_CH):
                if u1 <= _S_TRANS:
                    for cp in wr(u):
                        cp.start()
            rd(*_TAIL).wait()

        for u, (_, u1) in enumerate(_W_CH):
            if u1 in _WRITE_STEPS:
                @pl.when(s == u1)
                def _(u=u):
                    for cp in wr(u):
                        cp.start()

    def body(s, carry):
        a = lax.shift_right_logical(s, 5)
        b = lax.shift_right_logical(s, 4) & 1
        g0 = pl.multiple_of((s & (_SUB - 1)) * _GS, _GS)

        events = jnp.where(s < 32, _EVENTS_LO, _EVENTS_HI)

        @pl.when(lax.shift_right_logical(events, s & 31) & 1 == 1)
        def _():
            dma_bookkeeping(s)

        pv = pbuf[pl.ds(g0, _GS), a, b].reshape(n, C)
        q = jnp.dot(pv, wo[...], preferred_element_type=jnp.float32)
        for k in range(C // _LANE):
            qk = q[:, k * _LANE:(k + 1) * _LANE]
            up_ref[k, pl.ds(0, n, stride=2), :] = qk
            up_ref[k, pl.ds(1, n, stride=2), :] = qk
        up = jnp.concatenate([up_ref[k] for k in range(C // _LANE)], axis=1)
        up = up.reshape(_GS, 1, _BLK, C)

        cv = cbuf[pl.ds(g0, _GS), a, :, b].reshape(_GS * 2 * _BLK, C)
        acc = jnp.dot(cv, wc[...], preferred_element_type=jnp.float32)
        acc = acc.reshape(_GS, 2, _BLK, C)
        obuf[pl.ds(g0, _GS), a, :, b] = (acc + up).astype(obuf.dtype)
        return carry

    lax.fori_loop(0, _NS, body, 0)
    for cp in wr(len(_W_CH) - 1):
        cp.start()
    for u in range(len(_W_CH)):
        for cp in wr(u):
            cp.wait()


@jax.jit
def pallas_standalone__detection_seg_fpn_lateral__vision_kernel(
    c_fine: jax.Array,
    p_coarse: jax.Array,
    w_lat: jax.Array,
    w_out: jax.Array,
):
    Bn, H, W, C = c_fine.shape
    assert (Bn, H, W) == (1, _G * _A * 2, _B * _BLK) and C % _LANE == 0
    dt = c_fine.dtype
    fine = (_G, _A, 2, _B, _BLK, C)
    coarse = (_G, _A, _B, _BLK // 2, C)
    out = pl.pallas_call(
        _kernel,
        in_specs=[pl.BlockSpec(memory_space=pl.ANY)] * 4,
        out_specs=pl.BlockSpec(memory_space=pl.ANY),
        out_shape=jax.ShapeDtypeStruct(fine, dt),
        scratch_shapes=[
            pltpu.VMEM(fine, dt),
            pltpu.VMEM(coarse, dt),
            pltpu.VMEM(fine, dt),
            pltpu.VMEM((C, C), dt),
            pltpu.VMEM((C, C), dt),
            pltpu.VMEM((C, C), dt),
            pltpu.VMEM((C // _LANE, _GS * _BLK, _LANE), jnp.float32),
            pltpu.SemaphoreType.DMA((len(_C_CH),)),
            pltpu.SemaphoreType.DMA((len(_P_CH),)),
            pltpu.SemaphoreType.DMA((len(_W_CH), 2 * len(_W_SPLIT))),
            pltpu.SemaphoreType.DMA((2,)),
        ],
        compiler_params=pltpu.CompilerParams(
            vmem_limit_bytes=120 * 1024 * 1024),
    )(c_fine.reshape(fine), p_coarse.reshape(coarse), w_lat,
      w_out.reshape(C, C))
    return out.reshape(Bn, H, W, C)
```

```python
import jax
import jax.numpy as jnp
from jax import lax
import jax.experimental.pallas as pl
import jax.experimental.pallas.tpu as pltpu

_G = 64
_A = 2
_B = 2
_BLK = 128
_GS = 4
_SUB = _G // _GS
_NS = _A * _B * _SUB
_LANE = 128

_C_BOUNDS = (0, 1, 2, 4, 6, 10, 16, 24, 32, 48, 64)
_P_BOUNDS = (0, 2, 6, 16, 32, 48, 62, 64)
_W_BOUNDS = (0, 16, 32, 48, 59, 64)
_S_TRANS = 37
_W_SPLIT = (40, 48, 40)
_WC_CHUNKS = 2


def _pairs(b):
    return list(zip(b[:-1], b[1:]))


def _box(s0, s1):
    m = s0 // _SUB
    assert (s1 - 1) // _SUB == m
    return m, pl.ds((s0 % _SUB) * _GS, (s1 - s0) * _GS)


_C_CH = _pairs(_C_BOUNDS)
_P_CH = _pairs(_P_BOUNDS)
_W_CH = _pairs(_W_BOUNDS)
_READS = sorted(
    [("p", i, r) for i, r in enumerate(_P_CH[:-1])]
    + [("c", i, r) for i, r in enumerate(_C_CH)],
    key=lambda t: (t[2][0], t[0] != "p"))
_TAIL = ("p", len(_P_CH) - 1, _P_CH[-1])
_WAIT_STEPS = sorted({t[2][0] for t in _READS if t[2][0] < _S_TRANS})
_WRITE_STEPS = [u1 for _, u1 in _W_CH if _S_TRANS < u1 < _NS]
_EVENTS = sorted({*_WAIT_STEPS, _S_TRANS, *_WRITE_STEPS})
_EVENTS_LO = sum(1 << e for e in _EVENTS if e < 32)
_EVENTS_HI = sum(1 << (e - 32) for e in _EVENTS if e >= 32)
assert _NS <= 64 and max(_EVENTS_LO, _EVENTS_HI) < 2 ** 31
assert _SUB == 16 and _TAIL[2][0] >= _S_TRANS and sum(_W_SPLIT) == _BLK


def _kernel(c_hbm, p_hbm, wl_hbm, wo_hbm, o_hbm,
            cbuf, pbuf, obuf, wl, wo, wc, up_ref, csem, psem, osem, wsem):
    C = wl.shape[-1]
    n = _GS * _BLK // 2

    def rd(kind, i, r):
        m, g = _box(*r)
        a, b = divmod(m, _B)
        if kind == "c":
            return pltpu.make_async_copy(
                c_hbm.at[g, a, :, b], cbuf.at[m, g], csem.at[i])
        return pltpu.make_async_copy(
            p_hbm.at[g, a, b], pbuf.at[m, g], psem.at[i])

    def wr(u):
        m, g = _box(*_W_CH[u])
        a, b = divmod(m, _B)
        cps = []
        for par in range(2):
            r0 = 0
            for k, rows in enumerate(_W_SPLIT):
                r = pl.ds(r0, rows)
                cps.append(pltpu.make_async_copy(
                    obuf.at[m, g, par, r], o_hbm.at[g, a, par, b, r],
                    osem.at[u, par * len(_W_SPLIT) + k]))
                r0 += rows
        return cps

    wl_cp = pltpu.make_async_copy(wl_hbm, wl, wsem.at[0])
    wo_cp = pltpu.make_async_copy(wo_hbm, wo, wsem.at[1])
    wl_cp.start()
    wo_cp.start()
    for t in _READS + [_TAIL]:
        rd(*t).start()
    wl_cp.wait()
    wo_cp.wait()

    wc_rows = C // _WC_CHUNKS

    def wc_body(i, carry):
        rows = pl.ds(pl.multiple_of(i * wc_rows, wc_rows), wc_rows)
        wc[rows, :] = jnp.dot(
            wl[rows, :], wo[...],
            preferred_element_type=jnp.float32).astype(wc.dtype)
        return carry

    lax.fori_loop(0, _WC_CHUNKS, wc_body, 0)

    def dma_bookkeeping(s):
        for s0 in _WAIT_STEPS:
            @pl.when(s == s0)
            def _(s0=s0):
                for t in _READS:
                    if t[2][0] == s0:
                        rd(*t).wait()

        @pl.when(s == _S_TRANS)
        def _():
            for t in _READS:
                if t[2][0] >= _S_TRANS:
                    rd(*t).wait()
            for u, (_, u1) in enumerate(_W_CH):
                if u1 <= _S_TRANS:
                    for cp in wr(u):
                        cp.start()
            rd(*_TAIL).wait()

        for u, (_, u1) in enumerate(_W_CH):
            if u1 in _WRITE_STEPS:
                @pl.when(s == u1)
                def _(u=u):
                    for cp in wr(u):
                        cp.start()

    def body(s, carry):
        m = lax.shift_right_logical(s, 4)
        g = pl.ds(pl.multiple_of((s & (_SUB - 1)) * _GS, _GS), _GS)

        events = jnp.where(s < 32, _EVENTS_LO, _EVENTS_HI)

        @pl.when((lax.shift_right_logical(events, s & 31) & 1) == 1)
        def _():
            dma_bookkeeping(s)

        pv = pbuf[m, g].reshape(n, C)
        q = jnp.dot(pv, wo[...], preferred_element_type=jnp.float32)
        for k in range(C // _LANE):
            qk = q[:, k * _LANE:(k + 1) * _LANE]
            up_ref[k, pl.ds(0, n, stride=2), :] = qk
            up_ref[k, pl.ds(1, n, stride=2), :] = qk
        up = jnp.concatenate(
            [up_ref[k, pl.ds(0, 2 * n), :] for k in range(C // _LANE)], axis=1)
        up = up.reshape(_GS, 1, _BLK, C)

        cv = cbuf[m, g].reshape(_GS * 2 * _BLK, C)
        acc = jnp.dot(cv, wc[...], preferred_element_type=jnp.float32)
        acc = acc.reshape(_GS, 2, _BLK, C)
        obuf[m, g] = (acc + up).astype(obuf.dtype)
        return carry

    lax.fori_loop(0, _NS, body, 0)
    for cp in wr(len(_W_CH) - 1):
        cp.start()
    for u in range(len(_W_CH)):
        for cp in wr(u):
            cp.wait()


@jax.jit
def pallas_standalone__detection_seg_fpn_lateral__vision_kernel(
    c_fine: jax.Array,
    p_coarse: jax.Array,
    w_lat: jax.Array,
    w_out: jax.Array,
):
    Bn, H, W, C = c_fine.shape
    assert (Bn, H, W) == (1, _G * _A * 2, _B * _BLK) and C % _LANE == 0
    dt = c_fine.dtype
    fine = (_G, _A, 2, _B, _BLK, C)
    coarse = (_G, _A, _B, _BLK // 2, C)
    out = pl.pallas_call(
        _kernel,
        in_specs=[pl.BlockSpec(memory_space=pl.ANY)] * 4,
        out_specs=pl.BlockSpec(memory_space=pl.ANY),
        out_shape=jax.ShapeDtypeStruct(fine, dt),
        scratch_shapes=[
            pltpu.VMEM((_A * _B, _G, 2, _BLK, C), dt),
            pltpu.VMEM((_A * _B, _G, _BLK // 2, C), dt),
            pltpu.VMEM((_A * _B, _G, 2, _BLK, C), dt),
            pltpu.VMEM((C, C), dt),
            pltpu.VMEM((C, C), dt),
            pltpu.VMEM((C, C), dt),
            pltpu.VMEM((C // _LANE, _GS * _BLK + 8, _LANE), jnp.float32),
            pltpu.SemaphoreType.DMA((len(_C_CH),)),
            pltpu.SemaphoreType.DMA((len(_P_CH),)),
            pltpu.SemaphoreType.DMA((len(_W_CH), 2 * len(_W_SPLIT))),
            pltpu.SemaphoreType.DMA((2,)),
        ],
        compiler_params=pltpu.CompilerParams(
            vmem_limit_bytes=120 * 1024 * 1024),
    )(c_fine.reshape(fine), p_coarse.reshape(coarse), w_lat,
      w_out.reshape(C, C))
    return out.reshape(Bn, H, W, C)
```

```python
import jax
import jax.numpy as jnp
from jax import lax
import jax.experimental.pallas as pl
import jax.experimental.pallas.tpu as pltpu

_NR = 128
_FW = 256
_LANE = 128

_K = 16
_L = _NR // _K
_SPS = 2
_NS = _NR // _SPS

_GROUPS = (0, 2, 4, 8, 12, 16, 24, 32, 48, 64, 80, 128)
_TAIL = 4
_S_TRANS = 36
_WRITES = ((36, 64), (48, 96), (56, 112), (60, 120))
_W_SPLIT = (32, 48, 48) * 4
_WC_CHUNKS = 2


def _pieces(lo, hi):
    out = []
    for a in range(_L):
        k0, k1 = max(lo - a * _K, 0), min(hi - a * _K, _K)
        if k1 > k0:
            out.append((a, pl.ds(k0, k1 - k0), pl.ds(a * _K + k0, k1 - k0)))
    return out


_GR = list(zip(_GROUPS[:-1], _GROUPS[1:]))
_GR_STEP = [min(lo // _SPS, _S_TRANS) for lo, _ in _GR]
_WR = [(s, lo, hi) for (s, hi), lo
       in zip(_WRITES, (0,) + tuple(hi for _, hi in _WRITES))]
_EVENTS = sorted({*_GR_STEP, *(s for s, _ in _WRITES)})
_EVENTS_LO = sum(1 << e for e in _EVENTS if e < 32)
_EVENTS_HI = sum(1 << (e - 32) for e in _EVENTS if e >= 32)
assert _NS <= 64 and max(_EVENTS_LO, _EVENTS_HI) < 2 ** 31
assert sum(_W_SPLIT) == 2 * _FW and _WRITES[0][0] == _S_TRANS
assert _GROUPS[-2] < _NR - _TAIL and (_NR - _TAIL) // _SPS >= _S_TRANS
assert all(hi <= s * _SPS for s, hi in _WRITES)


def _kernel(c_hbm, p_hbm, wl_hbm, wo_hbm, o_hbm,
            cbuf, pbuf, obuf, wl, wo, wc, up_ref):
    C = wl.shape[-1]
    n = _SPS * _FW // 2

    def read(x_hbm, buf, lo, hi, sem):
        for a, k, slots in _pieces(lo, hi):
            pltpu.make_async_copy(x_hbm.at[k, a], buf.at[slots], sem).start()

    def wait(buf, lo, hi, sem):
        v = buf.at[pl.ds(lo, hi - lo)]
        pltpu.make_async_copy(v, v, sem).wait()

    def write(lo, hi, sem):
        for a, k, slots in _pieces(lo, hi):
            r0 = 0
            for rows in _W_SPLIT:
                r = pl.ds(r0, rows)
                pltpu.make_async_copy(
                    obuf.at[slots, r], o_hbm.at[k, a, r], sem).start()
                r0 += rows

    def main(rsem, osem):
        ng = len(_GR)
        tail = (_NR - _TAIL, _NR, rsem.at[2 * ng])
        wl_cp = pltpu.make_async_copy(wl_hbm, wl, rsem.at[2 * ng + 1])
        wo_cp = pltpu.make_async_copy(wo_hbm, wo, rsem.at[2 * ng + 2])
        wl_cp.start()
        wo_cp.start()
        for i, (lo, hi) in enumerate(_GR):
            read(p_hbm, pbuf, lo, min(hi, tail[0]), rsem.at[2 * i])
            read(c_hbm, cbuf, lo, hi, rsem.at[2 * i + 1])
        read(p_hbm, pbuf, *tail)
        wl_cp.wait()
        wo_cp.wait()

        wc_rows = C // _WC_CHUNKS

        def wc_body(i, carry):
            rows = pl.ds(pl.multiple_of(i * wc_rows, wc_rows), wc_rows)
            wc[rows, :] = jnp.dot(
                wl[rows, :], wo[...],
                preferred_element_type=jnp.float32).astype(wc.dtype)
            return carry

        lax.fori_loop(0, _WC_CHUNKS, wc_body, 0)

        def bookkeeping(e):
            for i, (lo, hi) in enumerate(_GR):
                if _GR_STEP[i] == e:
                    wait(pbuf, lo, min(hi, tail[0]), rsem.at[2 * i])
                    wait(cbuf, lo, hi, rsem.at[2 * i + 1])
            for s, lo, hi in _WR:
                if s == e:
                    write(lo, hi, osem)
            if e == _S_TRANS:
                wait(pbuf, *tail)

        def body(s, carry):
            events = jnp.where(s < 32, _EVENTS_LO, _EVENTS_HI)

            @pl.when((lax.shift_right_logical(events, s & 31) & 1) == 1)
            def _():
                for e in _EVENTS:
                    pl.when(s == e)(lambda e=e: bookkeeping(e))

            sl = pl.ds(pl.multiple_of(s * _SPS, _SPS), _SPS)
            q = jnp.dot(pbuf[sl].reshape(n, C), wo[...],
                        preferred_element_type=jnp.float32)
            for k in range(C // _LANE):
                qk = q[:, k * _LANE:(k + 1) * _LANE]
                up_ref[k, pl.ds(0, n, stride=2), :] = qk
                up_ref[k, pl.ds(1, n, stride=2), :] = qk
            up = jnp.concatenate(
                [up_ref[k, pl.ds(0, 2 * n), :] for k in range(C // _LANE)],
                axis=1).reshape(_SPS, 1, _FW, C)

            acc = jnp.dot(cbuf[sl].reshape(4 * n, C), wc[...],
                          preferred_element_type=jnp.float32)
            out = acc.reshape(_SPS, 2, _FW, C) + up
            obuf[sl] = out.astype(obuf.dtype).reshape(_SPS, 2 * _FW, C)
            return carry

        lax.fori_loop(0, _NS, body, 0)
        write(_WRITES[-1][1], _NR, osem)
        pltpu.make_async_copy(o_hbm, o_hbm, osem).wait()

    pl.run_scoped(main,
                  pltpu.SemaphoreType.DMA((2 * len(_GR) + 3,)),
                  pltpu.SemaphoreType.DMA(()))


@jax.jit
def pallas_standalone__detection_seg_fpn_lateral__vision_kernel(
    c_fine: jax.Array,
    p_coarse: jax.Array,
    w_lat: jax.Array,
    w_out: jax.Array,
):
    Bn, H, W, C = c_fine.shape
    assert (Bn, H, W) == (1, 2 * _NR, _FW) and C % _LANE == 0
    dt = c_fine.dtype
    out = pl.pallas_call(
        _kernel,
        in_specs=[pl.BlockSpec(memory_space=pl.ANY)] * 4,
        out_specs=pl.BlockSpec(memory_space=pl.ANY),
        out_shape=jax.ShapeDtypeStruct((_K, _L, 2 * _FW, C), dt),
        scratch_shapes=[
            pltpu.VMEM((_NR, 2 * _FW, C), dt),
            pltpu.VMEM((_NR, _FW // 2, C), dt),
            pltpu.VMEM((_NR, 2 * _FW, C), dt),
            pltpu.VMEM((C, C), dt),
            pltpu.VMEM((C, C), dt),
            pltpu.VMEM((C, C), dt),
            pltpu.VMEM((C // _LANE, _SPS * _FW + 8, _LANE), jnp.float32),
        ],
        compiler_params=pltpu.CompilerParams(
            vmem_limit_bytes=120 * 1024 * 1024),
    )(c_fine.reshape(_K, _L, 2 * _FW, C),
      p_coarse.reshape(_K, _L, _FW // 2, C),
      w_lat, w_out.reshape(C, C))
    return out.reshape(Bn, H, W, C)
```
